```python
import os as _os
_os.environ.setdefault("JAX_PLATFORMS", "cpu")
import jax
import jax.numpy as jnp

def _softmax(x, axis=-1):
    return jax.nn.softmax(x, axis=axis)
def _gelu(x):
    return jax.nn.gelu(x, approximate=True)
def _silu(x):
    return jax.nn.silu(x)
def _sigmoid(x):
    return jax.nn.sigmoid(x)
def _layernorm(x, axis=-1, eps=1e-5):
    m = jnp.mean(x, axis=axis, keepdims=True)
    v = jnp.var(x, axis=axis, keepdims=True)
    return (x - m) / jnp.sqrt(v + eps)
def _scatter_add(tgt, idx, src, axis=0):
    return tgt.at[idx].add(src)
def _segment_sum(src, seg, n):
    return jax.ops.segment_sum(src, seg, n)
class _Rng:
    def __init__(self, key):
        self._k = key
    def _next(self):
        self._k, sub = jax.random.split(self._k)
        return sub
    def normal(self, shape):
        return jax.random.normal(self._next(), shape, dtype=jnp.bfloat16)
    def randint(self, lo, hi, shape):
        return jax.random.randint(self._next(), shape, lo, hi, dtype=jnp.int32)
    def uniform(self, shape, lo=0.0, hi=1.0):
        return jax.random.uniform(self._next(), shape, jnp.bfloat16, lo, hi)
    def permutation(self, n):
        return jax.random.permutation(self._next(), n)


kernel_name = 'standalone__mha_softmax__near_ridge'

def setup_inputs():
    _rng = _Rng(jax.random.key(int.from_bytes(__import__("os").urandom(4), "little")))
    _w = (lambda a: (lambda t: t.astype(jnp.bfloat16) if jnp.issubdtype(t.dtype, jnp.floating) else t)(jnp.asarray(a)))
    B, H, Sq, Sk, D = 8, 32, 304, 2048, 128
    return {
        "q": _w((lambda *s: _rng.normal(s) * 0.4)(B, H, Sq, D)),
        "k": _w((lambda *s: _rng.normal(s) * 0.4)(B, H, Sk, D)),
        "v": _w((lambda *s: _rng.normal(s) * 0.05)(B, H, Sk, D)),
    }

def reference(q, k, v):
    scale = q.shape[-1] ** -0.5
    scores = jnp.einsum("bhqd,bhkd->bhqk", q, k) * scale
    p = _softmax(scores, axis=-1)
    return jnp.einsum("bhqk,bhkd->bhqd", p, v)
```

```python
import functools
import jax, jax.numpy as jnp
from jax import lax
import jax.experimental.pallas as pl
import jax.experimental.pallas.tpu as pltpu

C = 128 ** -0.5 * 1.4426950408889634
NT = (((1,), (1,)), ((), ()))
RD = {'XLA_TPU_RESCHEDULE_DMA_DONES': True}

def make(U=5, mode='full', vmem=100, GS=256, flags=RD, delta=9,
         tie_l=False, tie_acc=True, tie_out=4, newton=True, sep=True, NOB=2, ostart=1, extra=0, wg=6, sg=1, og=3):
    NS = U + extra
    def kern(q_hbm, k_hbm, v_hbm, o_hbm, q0buf, k0buf, obuf, s_scr, mx_scr, acc_scr, l_scr, z_scr,
             sems, so, s0, *bufs):
        N = q_hbm.shape[0]
        Sq, D = q_hbm.shape[1:]
        Sk = k_hbm.shape[1]
        NG = Sk // GS
        T = GS // 128
        R = Sq // 16
        assert (N - 1) % U == 0
        NI = (N - 1) // U
        do_dma = mode in ('full', 'dma')
        do_comp = mode in ('full', 'compute')
        if sep:
            qb = bufs[0:U]; kb = bufs[U:2 * U]; vb = bufs[2 * U:3 * U]
        else:
            qb = [bufs[0].at[u] for u in range(U)]; kb = [bufs[1].at[u] for u in range(U)]; vb = [bufs[2].at[u] for u in range(U)]

        def cq(h, u): return pltpu.make_async_copy(q_hbm.at[h], qb[u], sems.at[3 * u])
        def ck(h, u): return pltpu.make_async_copy(k_hbm.at[h], kb[u], sems.at[3 * u + 1])
        def cv(h, u): return pltpu.make_async_copy(v_hbm.at[h], vb[u], sems.at[3 * u + 2])
        def co(j, sl): return pltpu.make_async_copy(obuf.at[sl], o_hbm.at[pl.ds(j * U, U)], so.at[sl])

        z_scr[...] = jnp.zeros(z_scr.shape, jnp.int32)

        def fold16(x):
            b = pltpu.bitcast(x, jnp.int32).reshape(R, 16, 128)
            return (b[:, :8, :] | b[:, 8:, :]).reshape(R * 8, 128)

        def tie_rows(lhs, rows):
            rows = [r for r in rows if r is not None]
            if not rows:
                return lhs
            z = z_scr[...]
            d = rows[0]
            for r in rows[1:]: d = d | r
            d = d & jnp.concatenate([z] * R, axis=0)
            return pltpu.bitcast(pltpu.bitcast(lhs, jnp.int32) | d, jnp.bfloat16)

        def tie_f32(x, dep):
            zz = jnp.concatenate([z_scr[...]] * (Sq // 8), axis=0)
            return pltpu.bitcast(pltpu.bitcast(x, jnp.int32) | (pltpu.bitcast(dep, jnp.int32) & zz), jnp.float32)

        def rowmax(mx):
            return jnp.broadcast_to(jnp.max(mx, axis=-1, keepdims=True), (Sq, 128))

        def normalise(acc, lpart):
            l = jnp.sum(lpart, axis=-1, keepdims=True)
            if newton:
                r = pl.reciprocal(l, approx=True)
                r = r * (2.0 - l * r)
            else:
                r = 1.0 / l
            return (acc * r).astype(jnp.bfloat16)

        class AState:
            def __init__(self, qref, kref, S):
                self.q = qref[...]; self.kref = kref; self.S = S; self.mx = None; self.s = []
            def group(self, g, rows=()):
                k = self.kref[g * GS:(g + 1) * GS, :]
                q = tie_rows(self.q, rows)
                s = lax.dot_general(q, k, NT, preferred_element_type=jnp.float32)
                if self.S is not None:
                    self.S[:, g * GS:(g + 1) * GS] = s
                else:
                    self.s.append(s)
                for t in range(T):
                    st = s[:, t * 128:(t + 1) * 128]
                    self.mx = st if self.mx is None else jnp.maximum(self.mx, st)

        class BCState:
            def __init__(self, vref, S, m, svals=None):
                self.vref = vref; self.S = S; self.m = m; self.svals = svals
                self.l = None; self.acc = None; self.p = {}
            def B(self, g, dep=None):
                s = self.S[:, g * GS:(g + 1) * GS] if self.svals is None else self.svals[g]
                m = self.m if dep is None else tie_f32(self.m, dep)
                mb = jnp.concatenate([m] * T, axis=1) if T > 1 else m
                p = jnp.exp2((s - mb) * C)
                ts = [p[:, t * 128:(t + 1) * 128] for t in range(T)]
                while len(ts) > 1:
                    ts = [ts[i] + ts[i + 1] for i in range(0, len(ts), 2)]
                self.l = ts[0] if self.l is None else self.l + ts[0]
                self.p[g] = p.astype(jnp.bfloat16)
            def Cc(self, g):
                v = self.vref[g * GS:(g + 1) * GS, :]
                o = jnp.dot(self.p.pop(g), v, preferred_element_type=jnp.float32)
                self.acc = o if self.acc is None else self.acc + o

        def slot(qref, kref, vref, m, svals, last, pend, hooks=None):
            a = AState(qref, kref, s_scr if last else None)
            bc = BCState(vref, s_scr, m, svals)
            for g in range(NG):
                if hooks and g in hooks:
                    for hkf in hooks[g]: hkf()
                rows = []
                if tie_l and pend['l'] is not None: rows.append(fold16(pend['l']))
                if tie_acc and pend['acc'] is not None: rows.append(fold16(pend['acc']))
                for item in pend['outs']: item[0] -= 1
                for item in [it for it in pend['outs'] if it[0] <= 0]:
                    rows.append(item[1]); pend['outs'].remove(item)
                prevd = pend['prevd']
                a.group(g, rows)
                cur = a.mx
                if prevd is None:
                    dep = jnp.concatenate([jnp.zeros((delta * 16, 128), jnp.float32), cur[:Sq - delta * 16]], axis=0)
                else:
                    dep = jnp.concatenate([prevd[Sq - delta * 16:], cur[:Sq - delta * 16]], axis=0)
                bc.B(g, dep)
                pend['prevd'] = cur
                bc.Cc(g)
                pend['l'] = bc.l; pend['acc'] = bc.acc
            return a, bc

        if do_dma:
            c0 = [pltpu.make_async_copy(k_hbm.at[0], k0buf, sems.at[3 * U + 1]),
                  pltpu.make_async_copy(q_hbm.at[0], q0buf, sems.at[3 * U])]
            for c in c0: c.start()
            for u in range(U):
                ck(u + 1, u).start(); cq(u + 1, u).start(); cv(u, u).start()
            for c in c0: c.wait()
        if do_comp:
            a = AState(q0buf, k0buf, s_scr)
            for g in range(NG): a.group(g)
            mx_scr[...] = a.mx
            acc_scr[...] = jnp.zeros(acc_scr.shape, jnp.float32)
            l_scr[...] = jnp.ones(l_scr.shape, jnp.float32)

        def body(j, carry):
            h0 = j * U
            sl = lax.rem(j, NOB)
            pv = lax.rem(j + NOB - 1, NOB)
            pend = dict(l=None, acc=None, outs=[], prevd=None)
            def waits(u):
                h = h0 + u
                ck(h + 1, u).wait(); cq(h + 1, u).wait(); cv(h, u).wait()
            def refill(u, hh, guard=None):
                c1 = hh + 1 + U < N
                c2 = hh + U < N
                if guard is not None:
                    c1 = jnp.logical_and(guard, c1); c2 = jnp.logical_and(guard, c2)
                @pl.when(c1)
                def _():
                    ck(hh + 1 + U, u).start(); cq(hh + 1 + U, u).start()
                @pl.when(c2)
                def _():
                    cv(hh + U, u).start()
            def out_ops():
                @pl.when(j >= 1)
                def _(): co(j - 1, pv).start()
            def out_wait():
                @pl.when(j >= NOB)
                def _(): co(j - NOB, sl).wait()
            if do_dma:
                waits(0)
                out_wait()
            if do_comp:
                m = rowmax(mx_scr[...])
                out = normalise(acc_scr[...], l_scr[...])
                obuf[pv, U - 1] = out
                if tie_out: pend['outs'].append([tie_out, pltpu.bitcast(out, jnp.int32)])
            svals = None
            for u in range(U):
                h = h0 + u
                last = (u + 1 == U)
                hooks = {}
                if do_dma:
                    if u == 0:
                        hooks.setdefault(sg, []).append(functools.partial(refill, U - 1, h0 - 1, j >= 1))
                        hooks.setdefault(og, []).append(out_ops)
                    else:
                        hooks.setdefault(sg, []).append(functools.partial(refill, u - 1, h - 1))
                    if not last:
                        hooks.setdefault(wg, []).append(functools.partial(waits, u + 1))
                if do_comp:
                    a, bc = slot(qb[u], kb[u], vb[u], m, svals, last, pend, hooks)
                    svals = a.s
                    if not last:
                        m = rowmax(a.mx)
                        out = normalise(bc.acc, bc.l)
                        obuf[sl, u] = out
                        if tie_out: pend['outs'].append([tie_out, pltpu.bitcast(out, jnp.int32)])
                    else:
                        mx_scr[...] = a.mx
                        acc_scr[...] = bc.acc
                        l_scr[...] = bc.l
                else:
                    for g in sorted(hooks):
                        for hkf in hooks[g]: hkf()
            return carry

        lax.fori_loop(0, NI, body, 0)
        sl = (NI - 1) % NOB
        if do_comp:
            obuf[sl, U - 1] = normalise(acc_scr[...], l_scr[...])
        if do_dma:
            co(NI - 1, sl).start()
            cv(N - 1, 0).wait()
        if do_comp:
            bc = BCState(vb[0], s_scr, rowmax(mx_scr[...]))
            for g in range(NG):
                bc.B(g); bc.Cc(g)
            q0buf[...] = normalise(bc.acc, bc.l)
        cl = pltpu.make_async_copy(q0buf, o_hbm.at[N - 1], s0.at[0])
        cl.start()
        if do_dma:
            for jj in range(NI - NOB, NI):
                co(jj, jj % NOB).wait()
        cl.wait()

    @jax.jit
    def f(q, k, v):
        B, H, Sq, D = q.shape
        Sk = k.shape[2]
        q2 = q.reshape(B * H, Sq, D); k2 = k.reshape(B * H, Sk, D); v2 = v.reshape(B * H, Sk, D)
        cp = dict(vmem_limit_bytes=vmem * 1024 * 1024)
        if flags: cp['flags'] = flags
        if sep:
            bufs = [pltpu.VMEM((Sq, D), jnp.bfloat16)] * U + [pltpu.VMEM((Sk, D), jnp.bfloat16)] * (2 * U)
        else:
            bufs = [pltpu.VMEM((U, Sq, D), jnp.bfloat16), pltpu.VMEM((U, Sk, D), jnp.bfloat16), pltpu.VMEM((U, Sk, D), jnp.bfloat16)]
        out = pl.pallas_call(
            kern,
            in_specs=[pl.BlockSpec(memory_space=pl.ANY)] * 3,
            out_specs=pl.BlockSpec(memory_space=pl.ANY),
            out_shape=jax.ShapeDtypeStruct(q2.shape, q.dtype),
            scratch_shapes=[
                pltpu.VMEM((Sq, D), jnp.bfloat16),
                pltpu.VMEM((Sk, D), jnp.bfloat16),
                pltpu.VMEM((NOB, U, Sq, D), jnp.bfloat16),
                pltpu.VMEM((Sq, Sk), jnp.float32),
                pltpu.VMEM((Sq, 128), jnp.float32),
                pltpu.VMEM((Sq, 128), jnp.float32),
                pltpu.VMEM((Sq, 128), jnp.float32),
                pltpu.VMEM((8, 128), jnp.int32),
                pltpu.SemaphoreType.DMA((3 * U + 2,)),
                pltpu.SemaphoreType.DMA((NOB,)),
                pltpu.SemaphoreType.DMA((2,)),
            ] + bufs,
            compiler_params=pltpu.CompilerParams(**cp),
        )(q2, k2, v2)
        return out.reshape(q.shape)
    return f


_IMPL = make(U=5)


@jax.jit
def pallas_standalone__mha_softmax__near_ridge_kernel(q: jax.Array, k: jax.Array, v: jax.Array):
    return _IMPL(q, k, v)
```

```python
import functools
import jax, jax.numpy as jnp
from jax import lax
import jax.experimental.pallas as pl
import jax.experimental.pallas.tpu as pltpu

C = 128 ** -0.5 * 1.4426950408889634
NT = (((1,), (1,)), ((), ()))
RD = {'XLA_TPU_RESCHEDULE_DMA_DONES': True}

def make(U=5, mode='full', vmem=100, GS=256, flags=RD, delta=9, tie_l=False, tie_acc=True, tie_out=0,
         newton=True, NOB=2, nobc=True, ng=1, pace_norm=True, wkg=6, wvg=7, skg=7, svg=1, og=3, owg=0):
    def kern(q_hbm, k_hbm, v_hbm, o_hbm, q0buf, k0buf, obuf, s_scr, s0_scr, m_scr, mx_scr, acc_scr, l_scr, z_scr,
             sems, so, qb_, kb_, vb_):
        N = q_hbm.shape[0]
        Sq, D = q_hbm.shape[1:]
        Sk = k_hbm.shape[1]
        NG = Sk // GS
        T = GS // 128
        R = Sq // 16
        assert (N - 1) % U == 0 and U >= 3
        NI = (N - 1) // U
        do_dma = mode in ('full', 'dma')
        do_comp = mode in ('full', 'compute')
        qb = [qb_.at[u] for u in range(U)]; kb = [kb_.at[u] for u in range(U)]; vb = [vb_.at[u] for u in range(U)]

        def cq(h, u): return pltpu.make_async_copy(q_hbm.at[h], qb[u], sems.at[3 * u])
        def ck(h, u): return pltpu.make_async_copy(k_hbm.at[h], kb[u], sems.at[3 * u + 1])
        def cv(h, u): return pltpu.make_async_copy(v_hbm.at[h], vb[u], sems.at[3 * u + 2])
        def co(j, sl): return pltpu.make_async_copy(obuf.at[sl], o_hbm.at[pl.ds(j * U, U)], so.at[sl])

        z_scr[...] = jnp.zeros(z_scr.shape, jnp.int32)

        def fold16(x):
            b = pltpu.bitcast(x, jnp.int32).reshape(R, 16, 128)
            return (b[:, :8, :] | b[:, 8:, :]).reshape(R * 8, 128)

        def tie_rows(lhs, rows):
            rows = [r for r in rows if r is not None]
            if not rows:
                return lhs
            z = z_scr[...]
            d = rows[0]
            for r in rows[1:]: d = d | r
            d = d & jnp.concatenate([z] * R, axis=0)
            return pltpu.bitcast(pltpu.bitcast(lhs, jnp.int32) | d, jnp.bfloat16)

        def tie_f32(x, dep):
            zz = jnp.concatenate([z_scr[...]] * (Sq // 8), axis=0)
            return pltpu.bitcast(pltpu.bitcast(x, jnp.int32) | (pltpu.bitcast(dep, jnp.int32) & zz), jnp.float32)

        def rowmax(mx):
            return jnp.broadcast_to(jnp.max(mx, axis=-1, keepdims=True), (Sq, 128))

        def normalise(acc, lpart):
            l = jnp.sum(lpart, axis=-1, keepdims=True)
            if newton:
                r = pl.reciprocal(l, approx=True)
                r = r * (2.0 - l * r)
            else:
                r = 1.0 / l
            return (acc * r).astype(jnp.bfloat16)

        class AState:
            def __init__(self, qref, kref, store, mx=None):
                self.q = qref[...]; self.kref = kref; self.store = store; self.mx = mx
            def group(self, g, rows=()):
                k = self.kref[g * GS:(g + 1) * GS, :]
                q = tie_rows(self.q, rows)
                s = lax.dot_general(q, k, NT, preferred_element_type=jnp.float32)
                self.store(g, s)
                for t in range(T):
                    st = s[:, t * 128:(t + 1) * 128]
                    self.mx = st if self.mx is None else jnp.maximum(self.mx, st)

        class BCState:
            def __init__(self, vref, load, m):
                self.vref = vref; self.load = load; self.m = m
                self.l = None; self.acc = None
            def B(self, g, dep=None):
                s = self.load(g)
                m = self.m if dep is None else tie_f32(self.m, dep)
                mb = jnp.concatenate([m] * T, axis=1) if T > 1 else m
                p = jnp.exp2((s - mb) * C)
                ts = [p[:, t * 128:(t + 1) * 128] for t in range(T)]
                while len(ts) > 1:
                    ts = [ts[i] + ts[i + 1] for i in range(0, len(ts), 2)]
                self.l = ts[0] if self.l is None else self.l + ts[0]
                return p.astype(jnp.bfloat16)
            def Cc(self, g, p):
                v = self.vref[g * GS:(g + 1) * GS, :]
                o = jnp.dot(p, v, preferred_element_type=jnp.float32)
                self.acc = o if self.acc is None else self.acc + o

        def st_scr(g, s): s_scr[:, g * GS:(g + 1) * GS] = s
        def ld_scr(g): return s_scr[:, g * GS:(g + 1) * GS]
        def st_s0(g, s): s0_scr[...] = s

        if do_dma:
            c0 = [pltpu.make_async_copy(k_hbm.at[0], k0buf, sems.at[3 * U + 1]),
                  pltpu.make_async_copy(q_hbm.at[0], q0buf, sems.at[3 * U])]
            for c in c0: c.start()
            for u in range(U):
                ck(u + 1, u).start(); cq(u + 1, u).start(); cv(u, u).start()
            for c in c0: c.wait()
        if do_comp:
            a = AState(q0buf, k0buf, st_scr)
            for g in range(NG): a.group(g)
            m_scr[...] = rowmax(a.mx)
            acc_scr[...] = jnp.zeros(acc_scr.shape, jnp.float32)
            l_scr[...] = jnp.ones(l_scr.shape, jnp.float32)
        if do_dma:
            ck(1, 0).wait(); cq(1, 0).wait()
        if do_comp:
            a = AState(qb[0], kb[0], st_s0)
            a.group(0)
            mx_scr[...] = a.mx

        def body(j, carry):
            h0 = j * U
            sl = lax.rem(j, NOB)
            pv = lax.rem(j + NOB - 1, NOB)
            hooks = {}
            def hook(u, g, fn): hooks.setdefault((u, g), []).append(fn)
            if do_dma:
                def wait_kq(u):
                    def fn():
                        if u < U:
                            ck(h0 + u + 1, u).wait(); cq(h0 + u + 1, u).wait()
                        else:
                            @pl.when(h0 + U + 1 < N)
                            def _():
                                ck(h0 + U + 1, 0).wait(); cq(h0 + U + 1, 0).wait()
                    return fn
                def wait_v(u):
                    return lambda: cv(h0 + u, u).wait()
                def start_kq(u):
                    def fn():
                        @pl.when(h0 + u + 1 + U < N)
                        def _():
                            ck(h0 + u + 1 + U, u).start(); cq(h0 + u + 1 + U, u).start()
                    return fn
                def start_v(u):
                    def fn():
                        hh = h0 + u
                        cond = hh + U < N
                        if u < 0: cond = jnp.logical_and(j >= 1, cond)
                        @pl.when(cond)
                        def _():
                            cv(hh + U, u % U).start()
                    return fn
                def out_start():
                    @pl.when(j >= 1)
                    def _(): co(j - 1, pv).start()
                def out_wait():
                    @pl.when(j >= NOB)
                    def _(): co(j - NOB, sl).wait()
                for u in range(U):
                    hook(u, wkg, wait_kq(u + 1))
                    if u + 1 < U: hook(u, wvg, wait_v(u + 1))
                    hook(u, skg, start_kq(u))
                    hook(u, svg, start_v(u - 1))
                hook(0, og, out_start)
                cv(h0, 0).wait()
                if owg < 0: out_wait()
                else: hook(0, owg, out_wait)
            if not do_comp:
                for key in sorted(hooks):
                    for fn in hooks[key]: fn()
                return carry

            pend = dict(l=None, acc=None, outs=[], prevd=None)
            def st_prev(o): obuf[pv, U - 1] = o
            norms = [[ng, acc_scr[...], l_scr[...], st_prev]]
            m = m_scr[...]
            a = AState(qb[0], kb[0], None, mx_scr[...])
            a_vals = {}
            a.store = lambda g, s, d=a_vals: d.__setitem__(g, s)
            a_load = lambda g, d=a_vals: (s0_scr[...] if g == 0 else d[g])
            bc_load = ld_scr
            for u in range(U):
                last = (u + 1 == U)
                bc = BCState(vb[u], bc_load, m)
                for g in range(NG):
                    for fn in hooks.get((u, g), []): fn()
                    rows = []
                    if tie_l and pend['l'] is not None: rows.append(fold16(pend['l']))
                    if tie_acc and pend['acc'] is not None: rows.append(fold16(pend['acc']))
                    for item in pend['outs']: item[0] -= 1
                    for item in [it for it in pend['outs'] if it[0] <= 0]:
                        rows.append(item[1]); pend['outs'].remove(item)
                    prevd = pend['prevd']
                    ga = (g + 1) % NG
                    if ga == 0:
                        m_next = rowmax(a.mx)
                        done_vals, done_load = a_vals, a_load
                        nu = u + 1
                        a_vals = {}
                        if nu == U - 1:
                            a = AState(qb[nu], kb[nu], st_scr)
                            a_load = None
                        elif nu == U:
                            a = AState(qb[0], kb[0], st_s0)
                            a_load = None
                        else:
                            a = AState(qb[nu], kb[nu], lambda g, s, d=a_vals: d.__setitem__(g, s))
                            a_load = lambda g, d=a_vals: d[g]
                    a.group(ga, rows)
                    cur = a.mx
                    if prevd is None:
                        dep = jnp.concatenate([jnp.zeros((delta * 16, 128), jnp.float32), cur[:Sq - delta * 16]], axis=0)
                    else:
                        dep = jnp.concatenate([prevd[Sq - delta * 16:], cur[:Sq - delta * 16]], axis=0)
                    p = bc.B(g, dep)
                    pend['prevd'] = cur
                    bc.Cc(g, p)
                    pend['l'] = bc.l; pend['acc'] = bc.acc
                    for item in norms: item[0] -= 1
                    for item in [it for it in norms if it[0] < 0]:
                        lp = tie_f32(item[2], cur) if pace_norm else item[2]
                        out = normalise(item[1], lp)
                        item[3](out)
                        norms.remove(item)
                        if tie_out: pend['outs'].append([tie_out, pltpu.bitcast(out, jnp.int32)])
                if not last:
                    norms.append([ng, bc.acc, bc.l, lambda o, u=u: obuf.__setitem__((sl, u), o)])
                    m = m_next; bc_load = done_load
                else:
                    m_scr[...] = m_next
                    mx_scr[...] = a.mx
                    acc_scr[...] = bc.acc
                    l_scr[...] = bc.l
            assert not norms
            return carry

        lax.fori_loop(0, NI, body, 0)
        sl = (NI - 1) % NOB
        if do_comp:
            obuf[sl, U - 1] = normalise(acc_scr[...], l_scr[...])
        if do_dma:
            co(NI - 1, sl).start()
            cv(N - 1, 0).wait()
        if do_comp:
            bc = BCState(vb[0], ld_scr, m_scr[...])
            for g in range(NG):
                bc.Cc(g, bc.B(g))
            q0buf[...] = normalise(bc.acc, bc.l)
        cl = pltpu.make_async_copy(q0buf, o_hbm.at[N - 1], sems.at[3 * U])
        cl.start()
        if do_dma:
            for jj in range(NI - NOB, NI):
                co(jj, jj % NOB).wait()
        cl.wait()

    @jax.jit
    def f(q, k, v):
        B, H, Sq, D = q.shape
        Sk = k.shape[2]
        q2 = q.reshape(B * H, Sq, D); k2 = k.reshape(B * H, Sk, D); v2 = v.reshape(B * H, Sk, D)
        cp = dict(vmem_limit_bytes=vmem * 1024 * 1024)
        if flags: cp['flags'] = flags
        if nobc: cp['disable_bounds_checks'] = True
        out = pl.pallas_call(
            kern,
            in_specs=[pl.BlockSpec(memory_space=pl.ANY)] * 3,
            out_specs=pl.BlockSpec(memory_space=pl.ANY),
            out_shape=jax.ShapeDtypeStruct(q2.shape, q.dtype),
            scratch_shapes=[
                pltpu.VMEM((Sq, D), jnp.bfloat16),
                pltpu.VMEM((Sk, D), jnp.bfloat16),
                pltpu.VMEM((NOB, U, Sq, D), jnp.bfloat16),
                pltpu.VMEM((Sq, Sk), jnp.float32),
                pltpu.VMEM((Sq, GS), jnp.float32),
                pltpu.VMEM((Sq, 128), jnp.float32),
                pltpu.VMEM((Sq, 128), jnp.float32),
                pltpu.VMEM((Sq, 128), jnp.float32),
                pltpu.VMEM((Sq, 128), jnp.float32),
                pltpu.VMEM((8, 128), jnp.int32),
                pltpu.SemaphoreType.DMA((3 * U + 2,)),
                pltpu.SemaphoreType.DMA((NOB,)),
                pltpu.VMEM((U, Sq, D), jnp.bfloat16), pltpu.VMEM((U, Sk, D), jnp.bfloat16), pltpu.VMEM((U, Sk, D), jnp.bfloat16),
            ],
            compiler_params=pltpu.CompilerParams(**cp),
        )(q2, k2, v2)
        return out.reshape(q.shape)
    return f


_IMPL = make(U=15, tie_out=2)


@jax.jit
def pallas_standalone__mha_softmax__near_ridge_kernel(q: jax.Array, k: jax.Array, v: jax.Array):
    return _IMPL(q, k, v)
```

```python
import jax
import jax.numpy as jnp
from jax import lax
import jax.experimental.pallas as pl
import jax.experimental.pallas.tpu as pltpu

_LOG2E = 1.4426950408889634
_NT = (((1,), (1,)), ((), ()))

GS = 256
UNROLL = 17
DELTA = 10
NORM_AT = 0
TIE_OUT = 2
OUT_TAIL = 2
N_OBUF = 2
WAIT_AT, START_KQ_AT, START_V_AT = 7, 7, 2
OUT_B_AT, OUT_A_AT, OUT_WAIT_AT = 1, 1, 0


def _attention_kernel(q_hbm, k_hbm, v_hbm, o_hbm,
                      q0buf, k0buf, obuf, s_scr, s0_scr, m_scr, mx_scr, acc_scr, l_scr, z_scr,
                      sems, osems, buf):
    N, Sq, D = q_hbm.shape
    Sk = k_hbm.shape[1]
    U = UNROLL
    NG = Sk // GS
    T = GS // 128
    R = Sq // 16
    NI = (N - 1) // U
    UA = U - OUT_TAIL
    c = D ** -0.5 * _LOG2E

    kb = [buf.at[u, pl.ds(0, Sk)] for u in range(U)]
    vb = [buf.at[u, pl.ds(Sk, Sk)] for u in range(U)]
    qb = [buf.at[u, pl.ds(2 * Sk, Sq)] for u in range(U)]

    def cq(h, u, sem=None):
        return pltpu.make_async_copy(q_hbm.at[h], qb[u], sems.at[u if sem is None else sem])

    def ck(h, u, sem=None):
        return pltpu.make_async_copy(k_hbm.at[h], kb[u], sems.at[u if sem is None else sem])

    def cv(h, u):
        return pltpu.make_async_copy(v_hbm.at[h], vb[u], sems.at[u])

    def wait_slot(u):
        pltpu.make_async_copy(buf.at[u], buf.at[u], sems.at[u]).wait()

    def co_a(j, sl):
        return pltpu.make_async_copy(obuf.at[sl, pl.ds(0, UA)],
                                     o_hbm.at[pl.ds(j * U, UA)], osems.at[2 * sl])

    def co_b(j, sl):
        return pltpu.make_async_copy(obuf.at[sl, pl.ds(UA, OUT_TAIL)],
                                     o_hbm.at[pl.ds(j * U + UA, OUT_TAIL)], osems.at[2 * sl + 1])

    z_scr[...] = jnp.zeros(z_scr.shape, jnp.int32)

    def fold16(x):
        b = pltpu.bitcast(x, jnp.int32).reshape(R, 16, 128)
        return (b[:, :8, :] | b[:, 8:, :]).reshape(R * 8, 128)

    def tie_rows(lhs, deps):
        if not deps:
            return lhs
        d = deps[0]
        for t in deps[1:]:
            d = d | t
        d = d & jnp.concatenate([z_scr[...]] * R, axis=0)
        return pltpu.bitcast(pltpu.bitcast(lhs, jnp.int32) | d, jnp.bfloat16)

    def tie_f32(x, dep):
        zz = jnp.concatenate([z_scr[...]] * (Sq // 8), axis=0)
        return pltpu.bitcast(
            pltpu.bitcast(x, jnp.int32) | (pltpu.bitcast(dep, jnp.int32) & zz), jnp.float32)

    def rowmax(mx):
        return jnp.broadcast_to(jnp.max(mx, axis=-1, keepdims=True), (Sq, 128))

    def normalise(acc, lpart):
        l = jnp.sum(lpart, axis=-1, keepdims=True)
        r = pltpu.reciprocal(l, approx=True)
        r = r * (2.0 - l * r)
        return (acc * r).astype(jnp.bfloat16)

    class StageA:
        def __init__(self, qref, kref, store, mx=None):
            self.q = qref[...]
            self.kref = kref
            self.store = store
            self.mx = mx

        def group(self, g, deps=()):
            k = self.kref[g * GS:(g + 1) * GS, :]
            s = lax.dot_general(tie_rows(self.q, deps), k, _NT, preferred_element_type=jnp.float32)
            self.store(g, s)
            for t in range(T):
                st = s[:, t * 128:(t + 1) * 128]
                self.mx = st if self.mx is None else jnp.maximum(self.mx, st)

    class StageBC:
        def __init__(self, vref, load, m):
            self.vref = vref
            self.load = load
            self.m = m
            self.l = None
            self.acc = None

        def exp(self, g, dep=None):
            m = self.m if dep is None else tie_f32(self.m, dep)
            p = jnp.exp2((self.load(g) - jnp.concatenate([m] * T, axis=1)) * c)
            ts = [p[:, t * 128:(t + 1) * 128] for t in range(T)]
            while len(ts) > 1:
                ts = [ts[i] + ts[i + 1] for i in range(0, len(ts), 2)]
            self.l = ts[0] if self.l is None else self.l + ts[0]
            return p.astype(jnp.bfloat16)

        def pv(self, g, p):
            o = jnp.dot(p, self.vref[g * GS:(g + 1) * GS, :], preferred_element_type=jnp.float32)
            self.acc = o if self.acc is None else self.acc + o

    def st_scr(g, s):
        s_scr[:, g * GS:(g + 1) * GS] = s

    def ld_scr(g):
        return s_scr[:, g * GS:(g + 1) * GS]

    def st_s0(g, s):
        s0_scr[...] = s

    cq0 = pltpu.make_async_copy(q_hbm.at[0], q0buf, sems.at[U])
    ck0 = pltpu.make_async_copy(k_hbm.at[0], k0buf, sems.at[U + 1])
    cq0.start()
    ck0.start()
    ck(1, 0, U + 2).start()
    cq(1, 0, U + 3).start()
    cv(0, 0).start()
    for u in range(1, U):
        ck(u + 1, u).start()
        cq(u + 1, u).start()
        cv(u, u).start()
    cq0.wait()
    ck0.wait()
    a = StageA(q0buf, k0buf, st_scr)
    for g in range(NG):
        a.group(g)
    m_scr[...] = rowmax(a.mx)
    acc_scr[...] = jnp.zeros(acc_scr.shape, jnp.float32)
    l_scr[...] = jnp.ones(l_scr.shape, jnp.float32)
    ck(1, 0, U + 2).wait()
    cq(1, 0, U + 3).wait()
    a = StageA(qb[0], kb[0], st_s0)
    a.group(0)
    mx_scr[...] = a.mx
    cv(0, 0).wait()

    def body(j, carry):
        h0 = j * U
        sl = lax.rem(j, N_OBUF)
        pv = lax.rem(j + N_OBUF - 1, N_OBUF)

        hooks = {}

        def hook(u, g, fn):
            hooks.setdefault((u, g), []).append(fn)

        def wait_kq(u):
            if u < U:
                return lambda: wait_slot(u)
            return lambda: pl.when(h0 + U + 1 < N)(lambda: wait_slot(0))

        def start_kq(u):
            def go():
                ck(h0 + u + 1 + U, u).start()
                cq(h0 + u + 1 + U, u).start()
            return lambda: pl.when(h0 + u + 1 + U < N)(go)

        def start_v(u):
            def fn():
                cond = h0 + u + U < N
                if u < 0:
                    cond = jnp.logical_and(j >= 1, cond)
                pl.when(cond)(lambda: cv(h0 + u + U, u % U).start())
            return fn

        def out_wait():
            @pl.when(j >= N_OBUF)
            def _():
                co_a(j - N_OBUF, sl).wait()
                co_b(j - N_OBUF, sl).wait()

        for u in range(U):
            hook(u, WAIT_AT, wait_kq(u + 1))
            hook(u, START_KQ_AT, start_kq(u))
            hook(u, START_V_AT, start_v(u - 1))
        hook(0, OUT_B_AT, lambda: pl.when(j >= 1)(lambda: co_b(j - 1, pv).start()))
        hook(0, OUT_WAIT_AT, out_wait)
        hook(U - 1, OUT_A_AT, lambda: co_a(j, sl).start())

        def st_prev(o):
            obuf[pv, U - 1] = o

        norms = [[NORM_AT, acc_scr[...], l_scr[...], st_prev]]
        outs = []
        prev_mx = None
        prev_acc = None
        m = m_scr[...]
        vals = {}
        a = StageA(qb[0], kb[0], lambda g, s, d=vals: d.__setitem__(g, s), mx_scr[...])
        a_load = lambda g, d=vals: (s0_scr[...] if g == 0 else d[g])
        bc_load = ld_scr
        for u in range(U):
            last = u + 1 == U
            bc = StageBC(vb[u], bc_load, m)
            for g in range(NG):
                for fn in hooks.get((u, g), []):
                    fn()
                deps = []
                if prev_acc is not None:
                    deps.append(fold16(prev_acc))
                for item in outs:
                    item[0] -= 1
                for item in [it for it in outs if it[0] <= 0]:
                    deps.append(item[1])
                    outs.remove(item)
                ga = (g + 1) % NG
                if ga == 0:
                    m_next = rowmax(a.mx)
                    done_load = a_load
                    nu = u + 1
                    vals = {}
                    if nu == U - 1:
                        a, a_load = StageA(qb[nu], kb[nu], st_scr), None
                    elif nu == U:
                        a, a_load = StageA(qb[0], kb[0], st_s0), None
                    else:
                        a = StageA(qb[nu], kb[nu], lambda g, s, d=vals: d.__setitem__(g, s))
                        a_load = lambda g, d=vals: d[g]
                a.group(ga, deps)
                cur = a.mx
                head = jnp.zeros((DELTA * 16, 128), jnp.float32) if prev_mx is None \
                    else prev_mx[Sq - DELTA * 16:]
                p = bc.exp(g, jnp.concatenate([head, cur[:Sq - DELTA * 16]], axis=0))
                prev_mx = cur
                bc.pv(g, p)
                prev_acc = bc.acc
                for item in norms:
                    item[0] -= 1
                for item in [it for it in norms if it[0] < 0]:
                    out = normalise(item[1], tie_f32(item[2], cur))
                    item[3](out)
                    norms.remove(item)
                    outs.append([TIE_OUT, pltpu.bitcast(out, jnp.int32)])
            if not last:
                norms.append([NORM_AT, bc.acc, bc.l, lambda o, u=u: obuf.__setitem__((sl, u), o)])
                m = m_next
                bc_load = done_load
            else:
                m_scr[...] = m_next
                mx_scr[...] = a.mx
                acc_scr[...] = bc.acc
                l_scr[...] = bc.l
        return carry

    lax.fori_loop(0, NI, body, 0)

    sl = (NI - 1) % N_OBUF
    cv(N - 1, 0).wait()
    obuf[sl, U - 1] = normalise(acc_scr[...], l_scr[...])
    co_b(NI - 1, sl).start()
    bc = StageBC(vb[0], ld_scr, m_scr[...])
    for g in range(NG):
        bc.pv(g, bc.exp(g))
    q0buf[...] = normalise(bc.acc, bc.l)
    last_copy = pltpu.make_async_copy(q0buf, o_hbm.at[N - 1], sems.at[U])
    last_copy.start()
    for jj in range(NI - N_OBUF, NI):
        co_a(jj, jj % N_OBUF).wait()
        co_b(jj, jj % N_OBUF).wait()
    last_copy.wait()


@jax.jit
def pallas_standalone__mha_softmax__near_ridge_kernel(
    q: jax.Array,
    k: jax.Array,
    v: jax.Array,
):
    B, H, Sq, D = q.shape
    Sk = k.shape[2]
    N = B * H
    assert D == 128 and Sq % 16 == 0 and Sk % GS == 0
    assert (N - 1) % UNROLL == 0 and (N - 1) // UNROLL >= N_OBUF
    assert DELTA * 16 < Sq

    out = pl.pallas_call(
        _attention_kernel,
        in_specs=[pl.BlockSpec(memory_space=pl.ANY)] * 3,
        out_specs=pl.BlockSpec(memory_space=pl.ANY),
        out_shape=jax.ShapeDtypeStruct((N, Sq, D), q.dtype),
        scratch_shapes=[
            pltpu.VMEM((Sq, D), jnp.bfloat16),
            pltpu.VMEM((Sk, D), jnp.bfloat16),
            pltpu.VMEM((N_OBUF, UNROLL, Sq, D), jnp.bfloat16),
            pltpu.VMEM((Sq, Sk), jnp.float32),
            pltpu.VMEM((Sq, GS), jnp.float32),
            pltpu.VMEM((Sq, 128), jnp.float32),
            pltpu.VMEM((Sq, 128), jnp.float32),
            pltpu.VMEM((Sq, 128), jnp.float32),
            pltpu.VMEM((Sq, 128), jnp.float32),
            pltpu.VMEM((8, 128), jnp.int32),
            pltpu.SemaphoreType.DMA((UNROLL + 4,)),
            pltpu.SemaphoreType.DMA((2 * N_OBUF,)),
            pltpu.VMEM((UNROLL, 2 * Sk + Sq, D), jnp.bfloat16),
        ],
        compiler_params=pltpu.CompilerParams(
            vmem_limit_bytes=100 * 1024 * 1024,
            disable_bounds_checks=True,
            flags={"XLA_TPU_RESCHEDULE_DMA_DONES": True},
        ),
    )(q.reshape(N, Sq, D), k.reshape(N, Sk, D), v.reshape(N, Sk, D))
    return out.reshape(B, H, Sq, D)
```

```python
import jax
import jax.numpy as jnp
from jax import lax
import jax.experimental.pallas as pl
import jax.experimental.pallas.tpu as pltpu

_LOG2E = 1.4426950408889634
_NT = (((1,), (1,)), ((), ()))
_reciprocal = pltpu.reciprocal if hasattr(pltpu, "reciprocal") else pl.reciprocal

GS = 256
UNROLL = 17
DELTA = 10
NORM_AT = 0
TIE_OUT = 2
OUT_TAIL = 2
N_OBUF = 2
WAIT_AT, START_KQ_AT, START_V_AT = 7, 7, 2
OUT_B_AT, OUT_A_AT, OUT_WAIT_AT = 1, 1, 0


def _attention_kernel(q_hbm, k_hbm, v_hbm, o_hbm,
                      q0buf, obuf, s_scr, s0_scr, m_scr, mx_scr, acc_scr, l_scr, z_scr,
                      sems, osems, buf):
    N, Sq, D = q_hbm.shape
    Sk = k_hbm.shape[1]
    U = UNROLL
    NG = Sk // GS
    T = GS // 128
    R = Sq // 16
    NI = (N - 1) // U
    UA = U - OUT_TAIL
    c = D ** -0.5 * _LOG2E

    kb = [buf.at[u, pl.ds(0, Sk)] for u in range(U)]
    vb = [buf.at[u, pl.ds(Sk, Sk)] for u in range(U)]
    qb = [buf.at[u, pl.ds(2 * Sk, Sq)] for u in range(U)]

    def cq(h, u, sem=None):
        return pltpu.make_async_copy(q_hbm.at[h], qb[u], sems.at[u if sem is None else sem])

    def ck(h, u, sem=None):
        return pltpu.make_async_copy(k_hbm.at[h], kb[u], sems.at[u if sem is None else sem])

    def cv(h, u):
        return pltpu.make_async_copy(v_hbm.at[h], vb[u], sems.at[u])

    def wait_slot(u):
        pltpu.make_async_copy(buf.at[u], buf.at[u], sems.at[u]).wait()

    def co_a(j, sl):
        return pltpu.make_async_copy(obuf.at[sl, pl.ds(0, UA)],
                                     o_hbm.at[pl.ds(j * U, UA)], osems.at[2 * sl])

    def co_b(j, sl):
        return pltpu.make_async_copy(obuf.at[sl, pl.ds(UA, OUT_TAIL)],
                                     o_hbm.at[pl.ds(j * U + UA, OUT_TAIL)], osems.at[2 * sl + 1])

    z_scr[...] = jnp.zeros(z_scr.shape, jnp.int32)

    def fold16(x):
        b = pltpu.bitcast(x, jnp.int32).reshape(R, 16, 128)
        return (b[:, :8, :] | b[:, 8:, :]).reshape(R * 8, 128)

    def tie_rows(lhs, deps):
        if not deps:
            return lhs
        d = deps[0]
        for t in deps[1:]:
            d = d | t
        d = d & jnp.concatenate([z_scr[...]] * R, axis=0)
        return pltpu.bitcast(pltpu.bitcast(lhs, jnp.int32) | d, jnp.bfloat16)

    def tie_f32(x, dep):
        zz = jnp.concatenate([z_scr[...]] * (Sq // 8), axis=0)
        return pltpu.bitcast(
            pltpu.bitcast(x, jnp.int32) | (pltpu.bitcast(dep, jnp.int32) & zz), jnp.float32)

    def rowmax(mx):
        return jnp.broadcast_to(jnp.max(mx, axis=-1, keepdims=True), (Sq, 128))

    def normalise(acc, lpart):
        l = jnp.sum(lpart, axis=-1, keepdims=True)
        r = _reciprocal(l, approx=True)
        r = r * (2.0 - l * r)
        return (acc * r).astype(jnp.bfloat16)

    class StageA:
        def __init__(self, qref, kref, store, mx=None):
            self.q = qref[...]
            self.kref = kref
            self.store = store
            self.mx = mx

        def group(self, g, deps=()):
            k = self.kref[g * GS:(g + 1) * GS, :]
            s = lax.dot_general(tie_rows(self.q, deps), k, _NT, preferred_element_type=jnp.float32)
            self.store(g, s)
            for t in range(T):
                st = s[:, t * 128:(t + 1) * 128]
                self.mx = st if self.mx is None else jnp.maximum(self.mx, st)

    class StageBC:
        def __init__(self, vref, load, m):
            self.vref = vref
            self.load = load
            self.m = m
            self.l = None
            self.acc = None

        def exp(self, g, dep=None):
            m = self.m if dep is None else tie_f32(self.m, dep)
            p = jnp.exp2((self.load(g) - jnp.concatenate([m] * T, axis=1)) * c)
            ts = [p[:, t * 128:(t + 1) * 128] for t in range(T)]
            while len(ts) > 1:
                ts = [ts[i] + ts[i + 1] for i in range(0, len(ts), 2)]
            self.l = ts[0] if self.l is None else self.l + ts[0]
            return p.astype(jnp.bfloat16)

        def pv(self, g, p):
            o = jnp.dot(p, self.vref[g * GS:(g + 1) * GS, :], preferred_element_type=jnp.float32)
            self.acc = o if self.acc is None else self.acc + o

    def st_scr(g, s):
        s_scr[:, g * GS:(g + 1) * GS] = s

    def ld_scr(g):
        return s_scr[:, g * GS:(g + 1) * GS]

    def st_s0(g, s):
        s0_scr[...] = s

    cq0 = cq(0, U - 1, U)
    ck0 = ck(0, U - 1, U + 1)
    cq0.start()
    ck0.start()
    ck(1, 0, U + 2).start()
    cq(1, 0, U + 3).start()
    cv(0, 0).start()
    for u in range(1, U):
        if u < U - 1:
            ck(u + 1, u).start()
            cq(u + 1, u).start()
        cv(u, u).start()
    cq0.wait()
    ck0.wait()
    a = StageA(qb[U - 1], kb[U - 1], st_scr)
    for g in range(NG):
        a.group(g)
    ck(U, U - 1).start()
    cq(U, U - 1).start()
    m_scr[...] = rowmax(a.mx)
    acc_scr[...] = jnp.zeros(acc_scr.shape, jnp.float32)
    l_scr[...] = jnp.ones(l_scr.shape, jnp.float32)
    ck(1, 0, U + 2).wait()
    cq(1, 0, U + 3).wait()
    a = StageA(qb[0], kb[0], st_s0)
    a.group(0)
    mx_scr[...] = a.mx
    cv(0, 0).wait()

    def body(j, carry):
        h0 = j * U
        sl = lax.rem(j, N_OBUF)
        pv = lax.rem(j + N_OBUF - 1, N_OBUF)

        hooks = {}

        def hook(u, g, fn):
            hooks.setdefault((u, g), []).append(fn)

        def wait_kq(u):
            if u < U:
                return lambda: wait_slot(u)
            return lambda: pl.when(h0 + U + 1 < N)(lambda: wait_slot(0))

        def start_kq(u):
            def go():
                ck(h0 + u + 1 + U, u).start()
                cq(h0 + u + 1 + U, u).start()
            return lambda: pl.when(h0 + u + 1 + U < N)(go)

        def start_v(u):
            def fn():
                cond = h0 + u + U < N
                if u < 0:
                    cond = jnp.logical_and(j >= 1, cond)
                pl.when(cond)(lambda: cv(h0 + u + U, u % U).start())
            return fn

        def out_wait():
            @pl.when(j >= N_OBUF)
            def _():
                co_a(j - N_OBUF, sl).wait()
                co_b(j - N_OBUF, sl).wait()

        for u in range(U):
            hook(u, WAIT_AT, wait_kq(u + 1))
            hook(u, START_KQ_AT, start_kq(u))
            hook(u, START_V_AT, start_v(u - 1))
        hook(0, OUT_B_AT, lambda: pl.when(j >= 1)(lambda: co_b(j - 1, pv).start()))
        hook(0, OUT_WAIT_AT, out_wait)
        hook(U - 1, OUT_A_AT, lambda: co_a(j, sl).start())

        def st_prev(o):
            obuf[pv, U - 1] = o

        norms = [[NORM_AT, acc_scr[...], l_scr[...], st_prev]]
        outs = []
        prev_mx = None
        prev_acc = None
        m = m_scr[...]
        vals = {}
        a = StageA(qb[0], kb[0], lambda g, s, d=vals: d.__setitem__(g, s), mx_scr[...])
        a_load = lambda g, d=vals: (s0_scr[...] if g == 0 else d[g])
        bc_load = ld_scr
        for u in range(U):
            last = u + 1 == U
            bc = StageBC(vb[u], bc_load, m)
            for g in range(NG):
                for fn in hooks.get((u, g), []):
                    fn()
                deps = []
                if prev_acc is not None:
                    deps.append(fold16(prev_acc))
                for item in outs:
                    item[0] -= 1
                for item in [it for it in outs if it[0] <= 0]:
                    deps.append(item[1])
                    outs.remove(item)
                ga = (g + 1) % NG
                if ga == 0:
                    m_next = rowmax(a.mx)
                    done_load = a_load
                    nu = u + 1
                    vals = {}
                    if nu == U - 1:
                        a, a_load = StageA(qb[nu], kb[nu], st_scr), None
                    elif nu == U:
                        a, a_load = StageA(qb[0], kb[0], st_s0), None
                    else:
                        a = StageA(qb[nu], kb[nu], lambda g, s, d=vals: d.__setitem__(g, s))
                        a_load = lambda g, d=vals: d[g]
                a.group(ga, deps)
                cur = a.mx
                head = jnp.zeros((DELTA * 16, 128), jnp.float32) if prev_mx is None \
                    else prev_mx[Sq - DELTA * 16:]
                p = bc.exp(g, jnp.concatenate([head, cur[:Sq - DELTA * 16]], axis=0))
                prev_mx = cur
                bc.pv(g, p)
                prev_acc = bc.acc
                for item in norms:
                    item[0] -= 1
                for item in [it for it in norms if it[0] < 0]:
                    out = normalise(item[1], tie_f32(item[2], cur))
                    item[3](out)
                    norms.remove(item)
                    outs.append([TIE_OUT, pltpu.bitcast(out, jnp.int32)])
            if not last:
                norms.append([NORM_AT, bc.acc, bc.l, lambda o, u=u: obuf.__setitem__((sl, u), o)])
                m = m_next
                bc_load = done_load
            else:
                m_scr[...] = m_next
                mx_scr[...] = a.mx
                acc_scr[...] = bc.acc
                l_scr[...] = bc.l
        return carry

    lax.fori_loop(0, NI, body, 0)

    sl = (NI - 1) % N_OBUF
    cv(N - 1, 0).wait()
    obuf[sl, U - 1] = normalise(acc_scr[...], l_scr[...])
    co_b(NI - 1, sl).start()
    bc = StageBC(vb[0], ld_scr, m_scr[...])
    for g in range(NG):
        bc.pv(g, bc.exp(g))
    q0buf[...] = normalise(bc.acc, bc.l)
    last_copy = pltpu.make_async_copy(q0buf, o_hbm.at[N - 1], sems.at[U])
    last_copy.start()
    for jj in range(NI - N_OBUF, NI):
        co_a(jj, jj % N_OBUF).wait()
        co_b(jj, jj % N_OBUF).wait()
    last_copy.wait()


@jax.jit
def pallas_standalone__mha_softmax__near_ridge_kernel(
    q: jax.Array,
    k: jax.Array,
    v: jax.Array,
):
    B, H, Sq, D = q.shape
    Sk = k.shape[2]
    N = B * H
    assert D == 128 and Sq % 16 == 0 and Sk % GS == 0
    assert (N - 1) % UNROLL == 0 and (N - 1) // UNROLL >= N_OBUF
    assert DELTA * 16 < Sq

    out = pl.pallas_call(
        _attention_kernel,
        in_specs=[pl.BlockSpec(memory_space=pl.ANY)] * 3,
        out_specs=pl.BlockSpec(memory_space=pl.ANY),
        out_shape=jax.ShapeDtypeStruct((N, Sq, D), q.dtype),
        scratch_shapes=[
            pltpu.VMEM((Sq, D), jnp.bfloat16),
            pltpu.VMEM((N_OBUF, UNROLL, Sq, D), jnp.bfloat16),
            pltpu.VMEM((Sq, Sk), jnp.float32),
            pltpu.VMEM((Sq, GS), jnp.float32),
            pltpu.VMEM((Sq, 128), jnp.float32),
            pltpu.VMEM((Sq, 128), jnp.float32),
            pltpu.VMEM((Sq, 128), jnp.float32),
            pltpu.VMEM((Sq, 128), jnp.float32),
            pltpu.VMEM((8, 128), jnp.int32),
            pltpu.SemaphoreType.DMA((UNROLL + 4,)),
            pltpu.SemaphoreType.DMA((2 * N_OBUF,)),
            pltpu.VMEM((UNROLL, 2 * Sk + Sq, D), jnp.bfloat16),
        ],
        compiler_params=pltpu.CompilerParams(
            vmem_limit_bytes=100 * 1024 * 1024,
            disable_bounds_checks=True,
            flags={"XLA_TPU_RESCHEDULE_DMA_DONES": True},
        ),
    )(q.reshape(N, Sq, D), k.reshape(N, Sk, D), v.reshape(N, Sk, D))
    return out.reshape(B, H, Sq, D)
```
